```python
import os as _os
_os.environ.setdefault("JAX_PLATFORMS", "cpu")
import jax
import jax.numpy as jnp

def _softmax(x, axis=-1):
    return jax.nn.softmax(x, axis=axis)
def _gelu(x):
    return jax.nn.gelu(x, approximate=True)
def _silu(x):
    return jax.nn.silu(x)
def _sigmoid(x):
    return jax.nn.sigmoid(x)
def _layernorm(x, axis=-1, eps=1e-5):
    m = jnp.mean(x, axis=axis, keepdims=True)
    v = jnp.var(x, axis=axis, keepdims=True)
    return (x - m) / jnp.sqrt(v + eps)
def _scatter_add(tgt, idx, src, axis=0):
    return tgt.at[idx].add(src)
def _segment_sum(src, seg, n):
    return jax.ops.segment_sum(src, seg, n)
class _Rng:
    def __init__(self, key):
        self._k = key
    def _next(self):
        self._k, sub = jax.random.split(self._k)
        return sub
    def normal(self, shape):
        return jax.random.normal(self._next(), shape, dtype=jnp.bfloat16)
    def randint(self, lo, hi, shape):
        return jax.random.randint(self._next(), shape, lo, hi, dtype=jnp.int32)
    def uniform(self, shape, lo=0.0, hi=1.0):
        return jax.random.uniform(self._next(), shape, jnp.bfloat16, lo, hi)
    def permutation(self, n):
        return jax.random.permutation(self._next(), n)


kernel_name = 'sequential_preLN__mha_block__dense_activation_mish__prompt'

def setup_inputs():
    _rng = _Rng(jax.random.key(int.from_bytes(__import__("os").urandom(4), "little")))
    _w = (lambda a: (lambda t: t.astype(jnp.bfloat16) if jnp.issubdtype(t.dtype, jnp.floating) else t)(jnp.asarray(a)))
    def _A_setup():
        B, S, D, H = 1, 2048, 576, 32
        return {
            "x": _w((lambda *s: _rng.normal(s) * 0.05)(B, S, D)),
            "wqkv": _w((lambda *s: _rng.normal(s) * 0.05)(D, 3 * D)),
            "wo": _w((lambda *s: _rng.normal(s) * 0.05)(D, D)),
        }
    _A_in = _A_setup()

    def _B_setup():
        B, S, D, F = 1, 2048, 576, 4608
        return {
            "x": _w((lambda *s: _rng.normal(s) * 0.05)(B, S, D)),
            "w1": _w((lambda *s: _rng.normal(s) * 1.6)(D, F) * (D ** -0.5)),
            "b1": _w((lambda *s: _rng.normal(s) * 0.05)(F)),
            "w2": _w((lambda *s: _rng.normal(s) * 0.05)(F, D) * (F ** -0.5)),
        }
    _B_in = _B_setup()

    return {
        "A_x": _A_in["x"],
        "A_wqkv": _A_in["wqkv"],
        "A_wo": _A_in["wo"],
        "B_x": _B_in["x"],
        "B_w1": _B_in["w1"],
        "B_b1": _B_in["b1"],
        "B_w2": _B_in["w2"],
    }

def reference(A_x, A_wqkv, A_wo, B_x, B_w1, B_b1, B_w2):
    def _A_ref(x, wqkv, wo):
        B, S, D = x.shape
        H = 32
        Dh = D // H
        qkv = (lambda x, *d: x.transpose(*d))((x @ wqkv).reshape(B, S, 3, H, Dh), 2, 0, 3, 1, 4)
        q, k, v = qkv[0], qkv[1], qkv[2]
        scores = jnp.einsum("bhqd,bhkd->bhqk", q, k) * (Dh ** -0.5)
        p = _softmax(scores, axis=-1)
        o = jnp.einsum("bhqk,bhkd->bhqd", p, v)
        return (lambda x, *d: x.transpose(*d))(o, 0, 2, 1, 3).reshape(B, S, D) @ wo

    def _B_ref(x, w1, b1, w2):
        h = jnp.einsum("bsd,df->bsf", x, w1) + b1
        sp = jnp.log1p(jnp.exp(-jnp.abs(h))) + jnp.where(h > 0, h, jnp.zeros_like(h))
        act = h * jnp.tanh(sp)
        return jnp.einsum("bsf,fd->bsd", act, w2)

    x = A_x
    h = x + _A_ref(_layernorm(x, axis=-1), A_wqkv, A_wo)
    h2 = h + _B_ref(_layernorm(h, axis=-1), B_w1, B_b1, B_w2)
    return h2
```

```python
import functools
import math

import jax
import jax.numpy as jnp
from jax import lax
import jax.experimental.pallas as pl
import jax.experimental.pallas.tpu as pltpu

S = 2048
D = 576
H = 32
DH = 18
F = 4608
EPS = 1e-5
HPT = 7
NG = 5
LOG2E = math.log2(math.e)

P1_ROWS = 512
TS = 256
NS = S // TS
P3_ROWS = 512
FC = 256
OUT_ROWS = 512

NT_DIMS = (((1,), (1,)), ((), ()))


def _layernorm(xf):
    m = jnp.mean(xf, axis=-1, keepdims=True)
    xc = xf - m
    v = jnp.mean(xc * xc, axis=-1, keepdims=True)
    return xc * lax.rsqrt(v + EPS)


def _mish(hv):
    e = jnp.exp(jnp.minimum(hv, 20.0))
    n = e * (e + 2.0)
    return hv * (n / (n + 2.0))


def _kernel(x_hbm, wqkv_hbm, wo_hbm, w1_hbm, b1_hbm, w2_hbm, o_hbm,
            x_s, wqkv_s, wo_s, w1_s, b1_s, w2_s,
            wqk_s, wvt_s, q_s, k_s, vt_s, s0_s, s1_s, ot_s, h_s, xn_s, acc_s, out_s,
            in_sem, out_sem):
    f32, bf16 = jnp.float32, jnp.bfloat16

    cp_x = pltpu.make_async_copy(x_hbm, x_s, in_sem.at[0])
    cp_wqkv = pltpu.make_async_copy(wqkv_hbm, wqkv_s, in_sem.at[1])
    cp_wo = pltpu.make_async_copy(wo_hbm, wo_s, in_sem.at[2])
    cp_w1 = pltpu.make_async_copy(w1_hbm, w1_s, in_sem.at[3])
    cp_b1 = pltpu.make_async_copy(b1_hbm, b1_s, in_sem.at[4])
    cp_w2 = pltpu.make_async_copy(w2_hbm, w2_s, in_sem.at[5])
    cp_wqkv.start()
    cp_x.start()
    cp_wo.start()
    cp_b1.start()
    cp_w1.start()
    cp_w2.start()

    cp_wqkv.wait()
    for t in range(NG):
        c0 = HPT * DH * t
        wqk_s[:, 128 * t:128 * (t + 1)] = wqkv_s[:, c0:c0 + 128]
        wqk_s[:, 128 * (NG + t):128 * (NG + t + 1)] = wqkv_s[:, D + c0:D + c0 + 128]
    wvt_s[...] = wqkv_s[:, 2 * D:3 * D].astype(f32).T.astype(bf16)
    cp_x.wait()

    qscale = (DH ** -0.5) * LOG2E
    ones_rows = (lax.broadcasted_iota(jnp.int32, (8, P1_ROWS), 0) == 0).astype(f32)

    def p1_body(i, carry):
        r0 = pl.multiple_of(i * P1_ROWS, P1_ROWS)
        rows = pl.ds(r0, P1_ROWS)
        xn = _layernorm(x_s[rows, :].astype(f32)).astype(bf16)
        qk = jnp.dot(xn, wqk_s[...], preferred_element_type=f32)
        for t in range(NG):
            q_s[t, rows, :] = (qk[:, 128 * t:128 * (t + 1)] * qscale).astype(bf16)
            k_s[t, rows, :] = qk[:, 128 * (NG + t):128 * (NG + t + 1)].astype(bf16)
        vt = lax.dot_general(wvt_s[...], xn, NT_DIMS, preferred_element_type=f32)
        for hh in range(H):
            a = 8 * ((DH * hh) // 8)
            vt_s[hh, :, rows] = jnp.concatenate([vt[a:a + 24], ones_rows], axis=0).astype(bf16)
        return carry

    lax.fori_loop(0, S // P1_ROWS, p1_body, 0)

    def qk_sub(hq, u, s_out):
        g = hq // HPT
        j = hq - HPT * g
        lane = lax.broadcasted_iota(jnp.int32, (TS, 128), 1)
        msk = (lane >= j * DH) & (lane < j * DH + DH)
        q = q_s[g, u * TS:(u + 1) * TS, :]
        qh = jnp.where(msk, q, jnp.zeros_like(q))
        s = lax.dot_general(k_s[g], qh, NT_DIMS, preferred_element_type=f32)
        s_out[u] = s
        return jnp.max(s, axis=0, keepdims=True)

    def pv_sub(hp, u, s_in, m):
        p = jnp.exp2(s_in[u] - m).astype(bf16)
        o = jnp.dot(vt_s[hp], p, preferred_element_type=f32)
        on = o[0:24] * (1.0 / o[24:25])
        a = pl.multiple_of(8 * ((DH * hp) // 8), 8)
        r0 = DH * hp - a
        cols = slice(u * TS, (u + 1) * TS)
        row = lax.broadcasted_iota(jnp.int32, (8, TS), 0)
        first = jnp.where(row >= r0, on[0:8], ot_s[pl.ds(a, 8), cols])
        ot_s[pl.ds(a, 8), cols] = first
        ot_s[pl.ds(a + 8, 16), cols] = on[8:24]

    def stage(hq, s_out, hp, s_in, m_in):
        ms = []
        for u in range(NS):
            ms.append(qk_sub(hq, u, s_out))
            pv_sub(hp, u, s_in, m_in[:, u * TS:(u + 1) * TS])
        return jnp.concatenate(ms, axis=1)

    ot_s[0:8, :] = jnp.zeros((8, S), f32)
    m0 = jnp.concatenate([qk_sub(0, u, s0_s) for u in range(NS)], axis=1)

    def att_body(hh, m):
        return lax.cond(hh % 2 == 0,
                        lambda mm: stage(hh + 1, s1_s, hh, s0_s, mm),
                        lambda mm: stage(hh + 1, s0_s, hh, s1_s, mm), m)

    m_last = lax.fori_loop(0, H - 1, att_body, m0)
    for u in range(NS):
        pv_sub(H - 1, u, s1_s, m_last[:, u * TS:(u + 1) * TS])

    cp_wo.wait()

    def p3_body(i, carry):
        r0 = pl.multiple_of(i * P3_ROWS, P3_ROWS)
        rows = pl.ds(r0, P3_ROWS)
        o = ot_s[:, rows].T.astype(bf16)
        hv = x_s[rows, :].astype(f32) + jnp.dot(o, wo_s[...], preferred_element_type=f32)
        h_s[rows, :] = hv
        xn_s[rows, :] = _layernorm(hv).astype(bf16)
        return carry

    lax.fori_loop(0, S // P3_ROWS, p3_body, 0)

    cp_b1.wait()
    cp_w1.wait()
    cp_w2.wait()

    def ffn_chunk(c):
        c0 = pl.multiple_of(c * FC, FC)
        hid = jnp.dot(xn_s[...], w1_s[:, pl.ds(c0, FC)], preferred_element_type=f32)
        hid = hid + b1_s[:, pl.ds(c0, FC)].astype(f32)
        act = _mish(hid).astype(bf16)
        return jnp.dot(act, w2_s[pl.ds(c0, FC), :], preferred_element_type=f32)

    acc_s[...] = h_s[...]

    def p4_body(c, carry):
        acc_s[...] += ffn_chunk(c)
        return carry

    lax.fori_loop(0, F // FC, p4_body, 0)
    out_s[...] = acc_s[...].astype(bf16)
    cp_out = pltpu.make_async_copy(out_s, o_hbm, out_sem)
    cp_out.start()
    cp_out.wait()


@jax.jit
def pallas_sequential_preLN__mha_block__dense_activation_mish__prompt_kernel(
    A_x: jax.Array,
    A_wqkv: jax.Array,
    A_wo: jax.Array,
    B_x: jax.Array,
    B_w1: jax.Array,
    B_b1: jax.Array,
    B_w2: jax.Array,
):
    del B_x
    f32, bf16 = jnp.float32, jnp.bfloat16
    x2 = A_x.reshape(S, D)
    b1 = B_b1.reshape(1, F)
    any_spec = pl.BlockSpec(memory_space=pl.ANY)
    out = pl.pallas_call(
        _kernel,
        out_shape=jax.ShapeDtypeStruct((S, D), bf16),
        in_specs=[any_spec] * 6,
        out_specs=any_spec,
        scratch_shapes=[
            pltpu.VMEM((S, D), bf16),
            pltpu.VMEM((D, 3 * D), bf16),
            pltpu.VMEM((D, D), bf16),
            pltpu.VMEM((D, F), bf16),
            pltpu.VMEM((1, F), bf16),
            pltpu.VMEM((F, D), bf16),
            pltpu.VMEM((D, 2 * NG * 128), bf16),
            pltpu.VMEM((D, D), bf16),
            pltpu.VMEM((NG, S, 128), bf16),
            pltpu.VMEM((NG, S, 128), bf16),
            pltpu.VMEM((H, 32, S), bf16),
            pltpu.VMEM((NS, S, TS), f32),
            pltpu.VMEM((NS, S, TS), f32),
            pltpu.VMEM((D, S), f32),
            pltpu.VMEM((S, D), f32),
            pltpu.VMEM((S, D), bf16),
            pltpu.VMEM((S, D), f32),
            pltpu.VMEM((S, D), bf16),
            pltpu.SemaphoreType.DMA((6,)),
            pltpu.SemaphoreType.DMA(()),
        ],
        compiler_params=pltpu.CompilerParams(vmem_limit_bytes=110 * 1024 * 1024),
        name="preln_mha_mish_block",
    )(x2, A_wqkv, A_wo, B_w1, b1, B_w2)
    return out.reshape(1, S, D)
```

```python
import contextlib
import math
import os

import jax
import jax.numpy as jnp
from jax import lax
import jax.experimental.pallas as pl
import jax.experimental.pallas.tpu as pltpu

S = 2048
D = 576
H = 32
DH = 18
F = 4608
EPS = 1e-5
HPT = 7
NG = 5
LOG2E = math.log2(math.e)

P1 = 512
TS = 256
NS = S // TS
KV = int(os.environ.get("K_KV", "208"))
XW = int(os.environ.get("K_XW", "1"))
QS = int(os.environ.get("K_QS", "4"))
EPI = int(os.environ.get("K_EPI", "1"))
QG = int(os.environ.get("K_QG", "4"))
CH = int(os.environ.get("K_CH", "8"))
P3 = 512
FC = int(os.environ.get("K_FC", "512"))
OT = int(os.environ.get("K_OT", "128"))

NT_DIMS = (((1,), (1,)), ((), ()))
_SCOPES = os.environ.get("KERNEL_SCOPES", "") == "1"


def _scope(name):
    return jax.named_scope(name) if _SCOPES else contextlib.nullcontext()


def _layernorm_t(xf):
    m = jnp.sum(xf, axis=0, keepdims=True) * (1.0 / D)
    xc = xf - m
    v = jnp.sum(xc * xc, axis=0, keepdims=True) * (1.0 / D)
    return xc * lax.rsqrt(v + EPS)


def _mish(hv):
    e = jnp.exp(jnp.minimum(hv, 20.0))
    n = e * (e + 2.0)
    return hv * (n / (n + 2.0))


def _pack(v):
    return pltpu.bitcast(v, jnp.uint32)


def _unpack(v):
    return pltpu.bitcast(v, jnp.bfloat16)


def _kernel(x_hbm, wqkv_hbm, wo_hbm, w1_hbm, b1_hbm, w2t_hbm, o_hbm,
            x_s, wqkv_s, wo_s, w1_s, b1_s, w2t_s,
            wvt_s, wot_s, b1f_s, xnt_s, q_s, k_s, vt_s, qt_s, kf_s, kr0_s, kr1_s, qr0_s, qr1_s,
            s0_s, s1_s, ot_s, ht_s, xn_s, out_s,
            x_sem, w_sem, in_sem, out_sem, fence_sem):
    f32, bf16 = jnp.float32, jnp.bfloat16

    cp_xs = [pltpu.make_async_copy(x_hbm.at[:, i * P1:(i + 1) * P1], x_s.at[:, i * P1:(i + 1) * P1], x_sem.at[i])
             for i in range(S // P1)]
    w_cols = (0, 640, 2 * D, 3 * D)
    cp_wqkv = [pltpu.make_async_copy(wqkv_hbm.at[:, w_cols[i]:w_cols[i + 1]], wqkv_s.at[:, w_cols[i]:w_cols[i + 1]],
                                     w_sem.at[i]) for i in range(3)]
    cp_wo = pltpu.make_async_copy(wo_hbm, wo_s, in_sem.at[1])
    cp_b1 = pltpu.make_async_copy(b1_hbm, b1_s, in_sem.at[2])
    cp_w1 = pltpu.make_async_copy(w1_hbm, w1_s, in_sem.at[3])
    cp_w2 = pltpu.make_async_copy(w2t_hbm, w2t_s, in_sem.at[4])

    def fence():
        pl.semaphore_signal(fence_sem, 1)
        pl.semaphore_wait(fence_sem, 1)

    qk_scale = math.sqrt((DH ** -0.5) * LOG2E)
    ones_rows = (lax.broadcasted_iota(jnp.int32, (8, P1), 0) == 0).astype(f32)

    def ln1(i):
        toks = slice(i * P1, (i + 1) * P1)
        xnt_f = _layernorm_t(x_s[:, toks].astype(f32))
        xnt_s[:, toks] = _pack(xnt_f.astype(bf16))
        xn_s[i * P1 // 2:(i + 1) * P1 // 2, :] = _pack(xnt_f.T.astype(bf16))

    def proj_q(i):
        toks = slice(i * P1, (i + 1) * P1)
        half = slice(i * P1 // 2, (i + 1) * P1 // 2)
        qf = jnp.concatenate(
            [jnp.dot(_unpack(xn_s[(i * P1 + r) // 2:(i * P1 + r + P1 // QS) // 2, :]), wqkv_s[:, 0:640],
                     preferred_element_type=f32) for r in range(0, P1, P1 // QS)], axis=0) * qk_scale
        q = qf.astype(bf16)
        for t in range(NG):
            c0 = HPT * DH * t
            q_s[t, half, :] = _pack(q[:, c0:c0 + 128])
        qtf = qf[:, 0:D].T
        for hh in range(H):
            qt_s[hh, 0:DH, toks] = qtf[DH * hh:DH * (hh + 1)]
        return qf[:, 512:640]

    def proj_k(i, k_head):
        half = slice(i * P1 // 2, (i + 1) * P1 // 2)
        kf = jnp.dot(_unpack(xn_s[half, :]), wqkv_s[:, 640:2 * D], preferred_element_type=f32) * qk_scale
        kf = jnp.concatenate([k_head, kf], axis=1)
        k = kf.astype(bf16)
        for t in range(NG):
            c0 = 64 + HPT * DH * t
            if t < NG - 1:
                k_s[t, half, :] = _pack(k[:, c0:c0 + 128])
            else:
                k_s[t, half, :] = _pack(jnp.concatenate(
                    [k[:, c0:640], jnp.zeros((P1, 128 - (640 - c0)), bf16)], axis=1))
        if i == S // P1 - 1:
            for hh in range(H):
                kf_s[hh, :, 0:DH] = kf[P1 - KV:P1, 64 + DH * hh:64 + DH * (hh + 1)]

    def proj_v(i):
        toks = slice(i * P1, (i + 1) * P1)
        vt = jnp.dot(wvt_s[...], _unpack(xnt_s[:, toks]), preferred_element_type=f32)
        for hh in range(H):
            a = 8 * ((DH * hh) // 8)
            vt_s[hh, :, toks] = _pack(jnp.concatenate([vt[a:a + 24], ones_rows], axis=0).astype(bf16))

    with _scope("w_x0"):
        cp_xs[0].start()
        cp_wqkv[0].start()
        cp_xs[0].wait()
        cp_wqkv[1].start()
        cp_xs[1].start()
    with _scope("ln0"):
        ln1(0)
    with _scope("w_wq"):
        cp_wqkv[0].wait()
    with _scope("q0"):
        k_head = proj_q(0)
    with _scope("w_x1"):
        cp_wqkv[1].wait()
        cp_xs[1].wait()
        cp_wqkv[2].start()
        for cp in cp_xs[2:]:
            cp.start()
    with _scope("k0"):
        ln1(1)
        proj_k(0, k_head)
    with _scope("proj"):
        cp_wqkv[2].wait()
        for cp in cp_xs[2:]:
            cp.wait()
        cp_wo.start()
        cp_b1.start()
        cp_w1.start()
        cp_w2.start()
        wvt_s[...] = wqkv_s[:, 2 * D:3 * D].astype(f32).T.astype(bf16)
        for i in range(1, S // P1):
            if i > 1 and XW == 0:
                fence()
            if i + 1 < S // P1:
                ln1(i + 1)
            else:
                cp_wo.wait()
                wot_s[...] = wo_s[...].astype(f32).T.astype(bf16)
            proj_k(i, proj_q(i))
            proj_v(i - 1)
        proj_v(S // P1 - 1)

    def qk_mxu(hq, u, nkeys):
        g = hq // HPT
        j = hq - HPT * g
        lane = lax.broadcasted_iota(jnp.int32, (1, 128), 1)
        msk = jnp.where((lane >= j * DH) & (lane < j * DH + DH), jnp.uint32(0xFFFFFFFF), jnp.uint32(0))
        qh = _unpack(q_s[g, u * TS // 2:(u + 1) * TS // 2, :] & msk)
        return lax.dot_general(_unpack(k_s[g, 0:nkeys // 2, :]), qh, NT_DIMS, preferred_element_type=f32)

    def qk_sub0(u, s_out):
        s = qk_mxu(0, u, S)
        s_out[...] = s
        return jnp.max(s, axis=0, keepdims=True)

    KM = S - KV
    rep0, rep1 = (kr0_s, qr0_s), (kr1_s, qr1_s)

    def mk_krep(hq, kr, dds):
        kf = kf_s[hq, :, 0:DH]
        for dd in dds:
            kr[:, dd * 8:(dd + 1) * 8, :] = jnp.broadcast_to(kf[:, dd:dd + 1], (KV, 128)).reshape(KV // 8, 8, 128)

    def mk_qrep(hq, qr):
        for t in range(S // 128):
            qt = qt_s[hq, 0:DH, t * 128:(t + 1) * 128]
            for dd in range(DH):
                qr[t, dd * 8:(dd + 1) * 8, :] = jnp.broadcast_to(qt[dd:dd + 1], (8, 128))

    def qk_sub(hq, u, s_out, rep, rep_next):
        s = qk_mxu(hq, u, KM)
        s_out[0:KM, :] = s
        kr, qr = rep
        ntl = TS // 128
        qb = [[qr[u * ntl + t, dd * 8:(dd + 1) * 8, :] for dd in range(DH)] for t in range(ntl)]
        jobs = [(t, kg) for t in range(ntl) for kg in range(KV // 8)]
        nch = KM // CH
        mx = [None] * ntl
        done = 0
        side = {}
        if rep_next is not None:
            items = [(u * ntl + t, d0) for t in range(ntl) for d0 in range(0, DH, QG)]
            side = {(2 * n + 1) * nch // (2 * len(items)): it for n, it in enumerate(items)}
        for c in range(nch):
            cm = jnp.max(s[c * CH:(c + 1) * CH].reshape(CH // 8, 8, TS), axis=0)
            for t in range(ntl):
                ct = cm[:, t * 128:(t + 1) * 128]
                mx[t] = ct if mx[t] is None else jnp.maximum(mx[t], ct)
            if c in side:
                tt, d0 = side[c]
                g0 = 8 * (d0 // 8)
                g1 = min(g0 + 8, DH)
                qt = qt_s[hq + 1, g0:g1, tt * 128:(tt + 1) * 128]
                qt = jnp.maximum(qt, jnp.minimum(qt, mx[0][0:g1 - g0]))
                for dd in range(d0, min(d0 + QG, DH)):
                    rep_next[1][tt, dd * 8:(dd + 1) * 8, :] = jnp.broadcast_to(qt[dd - g0:dd - g0 + 1], (8, 128))
            upto = (len(jobs) * (c + 1) + nch // 2) // nch
            for (t, kg) in jobs[done:upto]:
                acc = None
                for dd in range(DH):
                    term = kr[kg, dd * 8:(dd + 1) * 8, :] * qb[t][dd]
                    acc = term if acc is None else acc + term
                s_out[KM + kg * 8:KM + (kg + 1) * 8, t * 128:(t + 1) * 128] = acc
                mx[t] = jnp.maximum(mx[t], acc)
            done = upto
        return jnp.max(jnp.concatenate(mx, axis=1), axis=0, keepdims=True)

    def pv_sub(hp, u, s_in, m):
        p = jnp.exp2(s_in[...] - m).astype(bf16)
        o = jnp.dot(_unpack(vt_s[hp]), p, preferred_element_type=f32)
        on = o[0:24] * (1.0 / o[24:25])
        a = 8 * ((DH * hp) // 8)
        r0 = DH * hp - a
        if not isinstance(a, int):
            a = pl.multiple_of(a, 8)
        cols = slice(u * TS, (u + 1) * TS)
        row = lax.broadcasted_iota(jnp.int32, (8, TS), 0)
        first = jnp.where(row >= r0, on[0:8], ot_s[pl.ds(a, 8), cols])
        ot_s[pl.ds(a, 8), cols] = first
        ot_s[pl.ds(a + 8, 16), cols] = on[8:24]

    def region(hp, s_in, s_out, rep_in, rep_out, ms):
        out = []
        for u in range(NS):
            out.append(qk_sub(hp + 1, u, s_out.at[u], rep_in, rep_out))
            pv_sub(hp, u, s_in.at[u], ms[u])
            if rep_out is not None:
                mk_krep(hp + 2, rep_out[0], range(u * DH // NS, (u + 1) * DH // NS))
        return tuple(out)

    with _scope("qk0"):
        ot_s[0:8, :] = jnp.zeros((8, S), f32)
        mk_krep(1, kr1_s, range(DH))
        mk_qrep(1, qr1_s)
        m0 = tuple(qk_sub0(u, s0_s.at[u]) for u in range(NS))

    def att_body(i, ms):
        ms = region(2 * i, s0_s, s1_s, rep1, rep0, ms)
        fence()
        return region(2 * i + 1, s1_s, s0_s, rep0, rep1, ms)

    with _scope("att"):
        ms = lax.fori_loop(0, (H - 2) // 2, att_body, m0)
        m_last = region(H - 2, s0_s, s1_s, rep1, None, ms)
        cp_b1.wait()
        cp_w1.wait()
        cp_w2.wait()
        b1f_s[...] = b1_s[...].astype(f32)

    KO = 512
    with _scope("epi"):
        for u in range(NS):
            cols = slice(u * TS, (u + 1) * TS)
            pv_sub(H - 1, u, s1_s.at[u], m_last[u])
            if EPI == 0:
                att = jnp.dot(wot_s[...], ot_s[:, cols].astype(bf16), preferred_element_type=f32)
            else:
                att = (jnp.dot(wot_s[:, 0:KO], ot_s[0:KO, cols].astype(bf16), preferred_element_type=f32)
                       + jnp.dot(wot_s[:, KO:D], ot_s[KO:D, cols].astype(bf16), preferred_element_type=f32))
            hv = x_s[:, cols].astype(f32) + att
            ht_s[:, cols] = hv
            xn_s[u * TS // 2:(u + 1) * TS // 2, :] = _pack(_layernorm_t(hv).T.astype(bf16))

    NC = F // FC

    def bias_row(c):
        return jnp.concatenate(
            [b1f_s[pl.ds(c * (FC // 128) + t, 1), :] for t in range(FC // 128)], axis=1)

    def ffn_act(c):
        c0 = c * FC
        if not isinstance(c0, int):
            c0 = pl.multiple_of(c0, FC)
        hid = jnp.dot(_unpack(xn_s[...]), w1_s[:, pl.ds(c0, FC)], preferred_element_type=f32)
        return _mish(hid + bias_row(c)).astype(bf16), w2t_s[:, pl.ds(c0, FC)]

    def ffn_step(c):
        act, w2c = ffn_act(c)
        ht_s[...] += lax.dot_general(w2c, act, NT_DIMS, preferred_element_type=f32)

    def out_copy(j):
        return pltpu.make_async_copy(out_s.at[:, j * OT:(j + 1) * OT], o_hbm.at[:, j * OT:(j + 1) * OT],
                                     out_sem.at[j])

    with _scope("ffn0"):
        ffn_step(0)

    with _scope("ffn"):
        def p4_body(c, carry):
            ffn_step(c)
            return carry

        lax.fori_loop(1, NC - 1, p4_body, 0)

    with _scope("ffn_last"):
        act, w2c = ffn_act(NC - 1)
        for j in range(S // OT):
            cols = slice(j * OT, (j + 1) * OT)
            fin = ht_s[:, cols] + lax.dot_general(w2c, act[cols], NT_DIMS, preferred_element_type=f32)
            out_s[:, cols] = fin.astype(bf16)
            out_copy(j).start()
        for j in range(S // OT):
            out_copy(j).wait()


@jax.jit
def pallas_sequential_preLN__mha_block__dense_activation_mish__prompt_kernel(
    A_x: jax.Array,
    A_wqkv: jax.Array,
    A_wo: jax.Array,
    B_x: jax.Array,
    B_w1: jax.Array,
    B_b1: jax.Array,
    B_w2: jax.Array,
):
    del B_x
    f32, bf16, u32 = jnp.float32, jnp.bfloat16, jnp.uint32
    xt = A_x.reshape(S, D).T
    w2t = B_w2.T
    b1 = B_b1.reshape(F // 128, 128)
    hbm_spec = pl.BlockSpec(memory_space=pltpu.HBM)
    out_t = pl.pallas_call(
        _kernel,
        out_shape=jax.ShapeDtypeStruct((D, S), bf16),
        in_specs=[hbm_spec] * 6,
        out_specs=hbm_spec,
        scratch_shapes=[
            pltpu.VMEM((D, S), bf16),
            pltpu.VMEM((D, 3 * D), bf16),
            pltpu.VMEM((D, D), bf16),
            pltpu.VMEM((D, F), bf16),
            pltpu.VMEM((F // 128, 128), bf16),
            pltpu.VMEM((D, F), bf16),
            pltpu.VMEM((D, D), bf16),
            pltpu.VMEM((D, D), bf16),
            pltpu.VMEM((F // 128, 128), f32),
            pltpu.VMEM((D // 2, S), u32),
            pltpu.VMEM((NG, S // 2, 128), u32),
            pltpu.VMEM((NG, S // 2, 128), u32),
            pltpu.VMEM((H, 16, S), u32),
            pltpu.VMEM((H, 24, S), f32),
            pltpu.VMEM((H, KV, 128), f32),
            pltpu.VMEM((KV // 8, DH * 8, 128), f32),
            pltpu.VMEM((KV // 8, DH * 8, 128), f32),
            pltpu.VMEM((S // 128, DH * 8, 128), f32),
            pltpu.VMEM((S // 128, DH * 8, 128), f32),
            pltpu.VMEM((NS, S, TS), f32),
            pltpu.VMEM((NS, S, TS), f32),
            pltpu.VMEM((D, S), f32),
            pltpu.VMEM((D, S), f32),
            pltpu.VMEM((S // 2, D), u32),
            pltpu.VMEM((D, S), bf16),
            pltpu.SemaphoreType.DMA((S // P1,)),
            pltpu.SemaphoreType.DMA((3,)),
            pltpu.SemaphoreType.DMA((5,)),
            pltpu.SemaphoreType.DMA((S // OT,)),
            pltpu.SemaphoreType.REGULAR,
        ],
        compiler_params=pltpu.CompilerParams(vmem_limit_bytes=124 * 1024 * 1024),
        name="preln_mha_mish_block",
    )(xt, A_wqkv, A_wo, B_w1, b1, w2t)
    return out_t.T.reshape(1, S, D)
```

```python
import math

import jax
import jax.numpy as jnp
from jax import lax
import jax.experimental.pallas as pl
import jax.experimental.pallas.tpu as pltpu

S = 2048
D = 576
H = 32
DH = 18
F = 4608
EPS = 1e-5
HPT = 7
NG = 5
LOG2E = math.log2(math.e)

P1 = 512
QS = 4
TS = 256
NS = S // TS
KV = 192
CH = 8
QG = 4
FC = 512
OT = 128

NT_DIMS = (((1,), (1,)), ((), ()))

def _layernorm_t(xf):
    m = jnp.sum(xf, axis=0, keepdims=True) * (1.0 / D)
    xc = xf - m
    v = jnp.sum(xc * xc, axis=0, keepdims=True) * (1.0 / D)
    return xc * lax.rsqrt(v + EPS)


def _mish(hv):
    e = jnp.exp(jnp.minimum(hv, 20.0))
    n = e * (e + 2.0)
    return hv * (n / (n + 2.0))


def _pack(v):
    return pltpu.bitcast(v, jnp.uint32)


def _unpack(v):
    return pltpu.bitcast(v, jnp.bfloat16)


def _kernel(x_hbm, wqkv_hbm, wo_hbm, w1_hbm, b1_hbm, w2t_hbm, o_hbm,
            x_s, wqkv_s, wo_s, w1_s, b1_s, w2t_s,
            wvt_s, wot_s, b1f_s, xnt_s, q_s, k_s, vt_s, qt_s, kf_s, kr0_s, kr1_s, qr0_s, qr1_s,
            s0_s, s1_s, ot_s, ht_s, xn_s, out_s,
            x_sem, w_sem, in_sem, out_sem, fence_sem):
    f32, bf16 = jnp.float32, jnp.bfloat16

    cp_xs = [pltpu.make_async_copy(x_hbm.at[:, i * P1:(i + 1) * P1], x_s.at[:, i * P1:(i + 1) * P1], x_sem.at[i])
             for i in range(S // P1)]
    w_cols = (0, 640, 2 * D, 3 * D)
    cp_wqkv = [pltpu.make_async_copy(wqkv_hbm.at[:, w_cols[i]:w_cols[i + 1]], wqkv_s.at[:, w_cols[i]:w_cols[i + 1]],
                                     w_sem.at[i]) for i in range(3)]
    cp_wo = pltpu.make_async_copy(wo_hbm, wo_s, in_sem.at[1])
    cp_b1 = pltpu.make_async_copy(b1_hbm, b1_s, in_sem.at[2])
    cp_w1 = pltpu.make_async_copy(w1_hbm, w1_s, in_sem.at[3])
    cp_w2 = pltpu.make_async_copy(w2t_hbm, w2t_s, in_sem.at[4])

    def fence():
        pl.semaphore_signal(fence_sem, 1)
        pl.semaphore_wait(fence_sem, 1)

    qk_scale = math.sqrt((DH ** -0.5) * LOG2E)
    ones_rows = (lax.broadcasted_iota(jnp.int32, (8, P1), 0) == 0).astype(f32)

    def ln1(i):
        toks = slice(i * P1, (i + 1) * P1)
        xnt_f = _layernorm_t(x_s[:, toks].astype(f32))
        xnt_s[:, toks] = _pack(xnt_f.astype(bf16))
        xn_s[i * P1 // 2:(i + 1) * P1 // 2, :] = _pack(xnt_f.T.astype(bf16))

    def proj_q(i):
        toks = slice(i * P1, (i + 1) * P1)
        half = slice(i * P1 // 2, (i + 1) * P1 // 2)
        qf = jnp.concatenate(
            [jnp.dot(_unpack(xn_s[(i * P1 + r) // 2:(i * P1 + r + P1 // QS) // 2, :]), wqkv_s[:, 0:640],
                     preferred_element_type=f32) for r in range(0, P1, P1 // QS)], axis=0) * qk_scale
        q = qf.astype(bf16)
        for t in range(NG):
            c0 = HPT * DH * t
            q_s[t, half, :] = _pack(q[:, c0:c0 + 128])
        qtf = qf[:, 0:D].T
        for hh in range(H):
            qt_s[hh, 0:DH, toks] = qtf[DH * hh:DH * (hh + 1)]
        return qf[:, 512:640]

    def proj_k(i, k_head):
        half = slice(i * P1 // 2, (i + 1) * P1 // 2)
        kf = jnp.dot(_unpack(xn_s[half, :]), wqkv_s[:, 640:2 * D], preferred_element_type=f32) * qk_scale
        kf = jnp.concatenate([k_head, kf], axis=1)
        k = kf.astype(bf16)
        for t in range(NG):
            c0 = 64 + HPT * DH * t
            if t < NG - 1:
                k_s[t, half, :] = _pack(k[:, c0:c0 + 128])
            else:
                k_s[t, half, :] = _pack(jnp.concatenate(
                    [k[:, c0:640], jnp.zeros((P1, 128 - (640 - c0)), bf16)], axis=1))
        if i == S // P1 - 1:
            for hh in range(H):
                kf_s[hh, :, 0:DH] = kf[P1 - KV:P1, 64 + DH * hh:64 + DH * (hh + 1)]

    def proj_v(i):
        toks = slice(i * P1, (i + 1) * P1)
        vt = jnp.dot(wvt_s[...], _unpack(xnt_s[:, toks]), preferred_element_type=f32)
        for hh in range(H):
            a = 8 * ((DH * hh) // 8)
            vt_s[hh, :, toks] = _pack(jnp.concatenate([vt[a:a + 24], ones_rows], axis=0).astype(bf16))

    cp_xs[0].start()
    cp_wqkv[0].start()
    cp_xs[0].wait()
    cp_wqkv[1].start()
    cp_xs[1].start()
    ln1(0)
    cp_wqkv[0].wait()
    k_head = proj_q(0)
    cp_wqkv[1].wait()
    cp_xs[1].wait()
    cp_wqkv[2].start()
    for cp in cp_xs[2:]:
        cp.start()
    ln1(1)
    proj_k(0, k_head)
    cp_wqkv[2].wait()
    for cp in cp_xs[2:]:
        cp.wait()
    cp_wo.start()
    cp_b1.start()
    cp_w1.start()
    cp_w2.start()
    wvt_s[...] = wqkv_s[:, 2 * D:3 * D].astype(f32).T.astype(bf16)
    for i in range(1, S // P1):
        if i + 1 < S // P1:
            ln1(i + 1)
        else:
            cp_wo.wait()
            wot_s[...] = wo_s[...].astype(f32).T.astype(bf16)
        proj_k(i, proj_q(i))
        proj_v(i - 1)
    proj_v(S // P1 - 1)

    def qk_mxu(hq, u, nkeys):
        g = hq // HPT
        j = hq - HPT * g
        lane = lax.broadcasted_iota(jnp.int32, (1, 128), 1)
        msk = jnp.where((lane >= j * DH) & (lane < j * DH + DH), jnp.uint32(0xFFFFFFFF), jnp.uint32(0))
        qh = _unpack(q_s[g, u * TS // 2:(u + 1) * TS // 2, :] & msk)
        return lax.dot_general(_unpack(k_s[g, 0:nkeys // 2, :]), qh, NT_DIMS, preferred_element_type=f32)

    def qk_sub0(u, s_out):
        s = qk_mxu(0, u, S)
        s_out[...] = s
        return jnp.max(s, axis=0, keepdims=True)

    KM = S - KV
    rep0, rep1 = (kr0_s, qr0_s), (kr1_s, qr1_s)

    def mk_krep(hq, kr, dds):
        kf = kf_s[hq, :, 0:DH]
        for dd in dds:
            kr[:, dd * 8:(dd + 1) * 8, :] = jnp.broadcast_to(kf[:, dd:dd + 1], (KV, 128)).reshape(KV // 8, 8, 128)

    def mk_qrep(hq, qr):
        for t in range(S // 128):
            qt = qt_s[hq, 0:DH, t * 128:(t + 1) * 128]
            for dd in range(DH):
                qr[t, dd * 8:(dd + 1) * 8, :] = jnp.broadcast_to(qt[dd:dd + 1], (8, 128))

    def qk_sub(hq, u, s_out, rep, rep_next):
        s = qk_mxu(hq, u, KM)
        s_out[0:KM, :] = s
        kr, qr = rep
        ntl = TS // 128
        qb = [[qr[u * ntl + t, dd * 8:(dd + 1) * 8, :] for dd in range(DH)] for t in range(ntl)]
        jobs = [(t, kg) for t in range(ntl) for kg in range(KV // 8)]
        nch = KM // CH
        mx = [None] * ntl
        done = 0
        side = {}
        if rep_next is not None:
            items = [(u * ntl + t, d0) for t in range(ntl) for d0 in range(0, DH, QG)]
            side = {(2 * n + 1) * nch // (2 * len(items)): it for n, it in enumerate(items)}
        for c in range(nch):
            cm = jnp.max(s[c * CH:(c + 1) * CH].reshape(CH // 8, 8, TS), axis=0)
            for t in range(ntl):
                ct = cm[:, t * 128:(t + 1) * 128]
                mx[t] = ct if mx[t] is None else jnp.maximum(mx[t], ct)
            if c in side:
                tt, d0 = side[c]
                g0 = 8 * (d0 // 8)
                g1 = min(g0 + 8, DH)
                qt = qt_s[hq + 1, g0:g1, tt * 128:(tt + 1) * 128]
                qt = jnp.maximum(qt, jnp.minimum(qt, mx[0][0:g1 - g0]))
                for dd in range(d0, min(d0 + QG, DH)):
                    rep_next[1][tt, dd * 8:(dd + 1) * 8, :] = jnp.broadcast_to(qt[dd - g0:dd - g0 + 1], (8, 128))
            upto = (len(jobs) * (c + 1) + nch // 2) // nch
            for (t, kg) in jobs[done:upto]:
                acc = None
                for dd in range(DH):
                    term = kr[kg, dd * 8:(dd + 1) * 8, :] * qb[t][dd]
                    acc = term if acc is None else acc + term
                s_out[KM + kg * 8:KM + (kg + 1) * 8, t * 128:(t + 1) * 128] = acc
                mx[t] = jnp.maximum(mx[t], acc)
            done = upto
        return jnp.max(jnp.concatenate(mx, axis=1), axis=0, keepdims=True)

    def pv_sub(hp, u, s_in, m):
        p = jnp.exp2(s_in[...] - m).astype(bf16)
        o = jnp.dot(_unpack(vt_s[hp]), p, preferred_element_type=f32)
        on = o[0:24] * (1.0 / o[24:25])
        a = 8 * ((DH * hp) // 8)
        r0 = DH * hp - a
        if not isinstance(a, int):
            a = pl.multiple_of(a, 8)
        cols = slice(u * TS, (u + 1) * TS)
        row = lax.broadcasted_iota(jnp.int32, (8, TS), 0)
        first = jnp.where(row >= r0, on[0:8], ot_s[pl.ds(a, 8), cols])
        ot_s[pl.ds(a, 8), cols] = first
        ot_s[pl.ds(a + 8, 16), cols] = on[8:24]

    def region(hp, s_in, s_out, rep_in, rep_out, ms):
        out = []
        for u in range(NS):
            out.append(qk_sub(hp + 1, u, s_out.at[u], rep_in, rep_out))
            pv_sub(hp, u, s_in.at[u], ms[u])
            if rep_out is not None:
                mk_krep(hp + 2, rep_out[0], range(u * DH // NS, (u + 1) * DH // NS))
        return tuple(out)

    ot_s[0:8, :] = jnp.zeros((8, S), f32)
    mk_krep(1, kr1_s, range(DH))
    mk_qrep(1, qr1_s)
    m0 = tuple(qk_sub0(u, s0_s.at[u]) for u in range(NS))

    def att_body(i, ms):
        ms = region(2 * i, s0_s, s1_s, rep1, rep0, ms)
        fence()
        return region(2 * i + 1, s1_s, s0_s, rep0, rep1, ms)

    ms = lax.fori_loop(0, (H - 2) // 2, att_body, m0)
    m_last = region(H - 2, s0_s, s1_s, rep1, None, ms)
    cp_b1.wait()
    cp_w1.wait()
    cp_w2.wait()
    b1f_s[...] = b1_s[...].astype(f32)

    KO = 512
    for u in range(NS):
        cols = slice(u * TS, (u + 1) * TS)
        pv_sub(H - 1, u, s1_s.at[u], m_last[u])
        att = (jnp.dot(wot_s[:, 0:KO], ot_s[0:KO, cols].astype(bf16), preferred_element_type=f32)
               + jnp.dot(wot_s[:, KO:D], ot_s[KO:D, cols].astype(bf16), preferred_element_type=f32))
        hv = x_s[:, cols].astype(f32) + att
        ht_s[:, cols] = hv
        xn_s[u * TS // 2:(u + 1) * TS // 2, :] = _pack(_layernorm_t(hv).T.astype(bf16))

    NC = F // FC

    def bias_row(c):
        return jnp.concatenate(
            [b1f_s[pl.ds(c * (FC // 128) + t, 1), :] for t in range(FC // 128)], axis=1)

    def ffn_act(c):
        c0 = c * FC
        if not isinstance(c0, int):
            c0 = pl.multiple_of(c0, FC)
        hid = jnp.dot(_unpack(xn_s[...]), w1_s[:, pl.ds(c0, FC)], preferred_element_type=f32)
        return _mish(hid + bias_row(c)).astype(bf16), w2t_s[:, pl.ds(c0, FC)]

    def ffn_step(c):
        act, w2c = ffn_act(c)
        ht_s[...] += lax.dot_general(w2c, act, NT_DIMS, preferred_element_type=f32)

    def out_copy(j):
        return pltpu.make_async_copy(out_s.at[:, j * OT:(j + 1) * OT], o_hbm.at[:, j * OT:(j + 1) * OT],
                                     out_sem.at[j])

    ffn_step(0)

    def p4_body(c, carry):
        ffn_step(c)
        return carry

    lax.fori_loop(1, NC - 1, p4_body, 0)

    act, w2c = ffn_act(NC - 1)
    for j in range(S // OT):
        cols = slice(j * OT, (j + 1) * OT)
        fin = ht_s[:, cols] + lax.dot_general(w2c, act[cols], NT_DIMS, preferred_element_type=f32)
        out_s[:, cols] = fin.astype(bf16)
        out_copy(j).start()
    for j in range(S // OT):
        out_copy(j).wait()


@jax.jit
def pallas_sequential_preLN__mha_block__dense_activation_mish__prompt_kernel(
    A_x: jax.Array,
    A_wqkv: jax.Array,
    A_wo: jax.Array,
    B_x: jax.Array,
    B_w1: jax.Array,
    B_b1: jax.Array,
    B_w2: jax.Array,
):
    del B_x
    f32, bf16, u32 = jnp.float32, jnp.bfloat16, jnp.uint32
    xt = A_x.reshape(S, D).T
    w2t = B_w2.T
    b1 = B_b1.reshape(F // 128, 128)
    hbm_spec = pl.BlockSpec(memory_space=pltpu.HBM)
    out_t = pl.pallas_call(
        _kernel,
        out_shape=jax.ShapeDtypeStruct((D, S), bf16),
        in_specs=[hbm_spec] * 6,
        out_specs=hbm_spec,
        scratch_shapes=[
            pltpu.VMEM((D, S), bf16),
            pltpu.VMEM((D, 3 * D), bf16),
            pltpu.VMEM((D, D), bf16),
            pltpu.VMEM((D, F), bf16),
            pltpu.VMEM((F // 128, 128), bf16),
            pltpu.VMEM((D, F), bf16),
            pltpu.VMEM((D, D), bf16),
            pltpu.VMEM((D, D), bf16),
            pltpu.VMEM((F // 128, 128), f32),
            pltpu.VMEM((D // 2, S), u32),
            pltpu.VMEM((NG, S // 2, 128), u32),
            pltpu.VMEM((NG, S // 2, 128), u32),
            pltpu.VMEM((H, 16, S), u32),
            pltpu.VMEM((H, 24, S), f32),
            pltpu.VMEM((H, KV, 128), f32),
            pltpu.VMEM((KV // 8, DH * 8, 128), f32),
            pltpu.VMEM((KV // 8, DH * 8, 128), f32),
            pltpu.VMEM((S // 128, DH * 8, 128), f32),
            pltpu.VMEM((S // 128, DH * 8, 128), f32),
            pltpu.VMEM((NS, S, TS), f32),
            pltpu.VMEM((NS, S, TS), f32),
            pltpu.VMEM((D, S), f32),
            pltpu.VMEM((D, S), f32),
            pltpu.VMEM((S // 2, D), u32),
            pltpu.VMEM((D, S), bf16),
            pltpu.SemaphoreType.DMA((S // P1,)),
            pltpu.SemaphoreType.DMA((3,)),
            pltpu.SemaphoreType.DMA((5,)),
            pltpu.SemaphoreType.DMA((S // OT,)),
            pltpu.SemaphoreType.REGULAR,
        ],
        compiler_params=pltpu.CompilerParams(
            vmem_limit_bytes=124 * 1024 * 1024,
            flags={"XLA_TPU_EVENLY_DISTRIBUTE_CRITICAL_NODES": True}),
        name="preln_mha_mish_block",
    )(xt, A_wqkv, A_wo, B_w1, b1, w2t)
    return out_t.T.reshape(1, S, D)
```
